```python
import os as _os
_os.environ.setdefault("JAX_PLATFORMS", "cpu")
import jax
import jax.numpy as jnp

def _softmax(x, axis=-1):
    return jax.nn.softmax(x, axis=axis)
def _gelu(x):
    return jax.nn.gelu(x, approximate=True)
def _silu(x):
    return jax.nn.silu(x)
def _sigmoid(x):
    return jax.nn.sigmoid(x)
def _layernorm(x, axis=-1, eps=1e-5):
    m = jnp.mean(x, axis=axis, keepdims=True)
    v = jnp.var(x, axis=axis, keepdims=True)
    return (x - m) / jnp.sqrt(v + eps)
def _scatter_add(tgt, idx, src, axis=0):
    return tgt.at[idx].add(src)
def _segment_sum(src, seg, n):
    return jax.ops.segment_sum(src, seg, n)
class _Rng:
    def __init__(self, key):
        self._k = key
    def _next(self):
        self._k, sub = jax.random.split(self._k)
        return sub
    def normal(self, shape):
        return jax.random.normal(self._next(), shape, dtype=jnp.bfloat16)
    def randint(self, lo, hi, shape):
        return jax.random.randint(self._next(), shape, lo, hi, dtype=jnp.int32)
    def uniform(self, shape, lo=0.0, hi=1.0):
        return jax.random.uniform(self._next(), shape, jnp.bfloat16, lo, hi)
    def permutation(self, n):
        return jax.random.permutation(self._next(), n)


kernel_name = 'parallel_sum__softmax_full_mha__swiglu_ffn__prompt'

def setup_inputs():
    _rng = _Rng(jax.random.key(int.from_bytes(__import__("os").urandom(4), "little")))
    _w = (lambda a: (lambda t: t.astype(jnp.bfloat16) if jnp.issubdtype(t.dtype, jnp.floating) else t)(jnp.asarray(a)))
    def _A_setup():
        B, S, D = 1, 2048, 640
        return {
            "x": _w((lambda *s: _rng.normal(s) * 0.05)(B, S, D)),
            "wqkv": _w((lambda *s: _rng.normal(s) * 0.1)(D, 3 * D)),
            "wo": _w((lambda *s: _rng.normal(s) * 0.05)(D, D)),
        }
    _A_in = _A_setup()

    def _B_setup():
        B, S, D, F = 1, 2048, 640, 1536
        return {
            "x": _w((lambda *s: _rng.normal(s) * 0.05)(B, S, D)),
            "w_gate": _w((lambda *s: _rng.normal(s) * 0.05)(D, F)),
            "w_up": _w((lambda *s: _rng.normal(s) * 0.05)(D, F)),
            "w_down": _w((lambda *s: _rng.normal(s) * 0.05)(F, D)),
        }
    _B_in = _B_setup()

    return {
        "A_x": _A_in["x"],
        "A_wqkv": _A_in["wqkv"],
        "A_wo": _A_in["wo"],
        "B_x": _B_in["x"],
        "B_w_gate": _B_in["w_gate"],
        "B_w_up": _B_in["w_up"],
        "B_w_down": _B_in["w_down"],
    }

def reference(A_x, A_wqkv, A_wo, B_x, B_w_gate, B_w_up, B_w_down):
    def _A_ref(x, wqkv, wo):
        B, S, D = x.shape
        H = 32; Dh = D // H
        qkv = (lambda x, *d: x.transpose(*d))((x @ wqkv).reshape(B, S, 3, H, Dh), 2, 0, 3, 1, 4)
        q, k, v = qkv[0], qkv[1], qkv[2]
        scale = Dh ** -0.5
        scores = jnp.einsum("bhqd,bhkd->bhqk", q, k) * scale
        p = _softmax(scores, axis=-1)
        o = jnp.einsum("bhqk,bhkd->bhqd", p, v)
        return (lambda x, *d: x.transpose(*d))(o, 0, 2, 1, 3).reshape(B, S, D) @ wo

    def _B_ref(x, w_gate, w_up, w_down):
        g = _silu(x @ w_gate)
        u = x @ w_up
        return (g * u) @ w_down

    x = A_x
    xn = _layernorm(x, axis=-1)
    return x + _A_ref(xn, A_wqkv, A_wo) + _B_ref(xn, B_w_gate, B_w_up, B_w_down)
```

```python
import functools, math
import jax
import jax.numpy as jnp
import jax.experimental.pallas as pl
import jax.experimental.pallas.tpu as pltpu

S, D, F = 2048, 640, 1536
H, DH = 32, 20
VR = 24
NG = D // 128
NT_DIMS = (((1,), (1,)), ((), ()))
QSCALE = (DH ** -0.5) * math.log2(math.e)
F32 = jnp.float32
BF16 = jnp.bfloat16


def make_kernel(TQ=512, CK=128, RC=512, NS=6, LAG=1, FR=512, PBF=1, SC=128):
    NQ = S // TQ
    NU = H * NQ
    NC = S // CK
    NR = S // RC
    NFR = S // FR
    n_iter = (NU - 2) // NS
    assert n_iter * NS == NU - 2 and NS % 2 == 0

    def kernel(x_hbm, wqkv_hbm, wo_hbm, wg_hbm, wu_hbm, wd_hbm, out_hbm,
               x_ref, wqkv_ref, wo_ref, wg_ref, wu_ref, wd_ref, o_ref,
               xn_ref, q_ref, k_ref, vt_ref, ot_ref, sa_ref, sb_ref, wt_ref, z_ref, sems):
        def x_copy(r):
            return pltpu.make_async_copy(x_hbm.at[pl.ds(r * RC, RC), :], x_ref.at[pl.ds(r * RC, RC), :], sems.at[r])

        def w_copy(i):
            return pltpu.make_async_copy(wqkv_hbm.at[:, pl.ds(i * D, D)], wqkv_ref.at[:, pl.ds(i * D, D)], sems.at[NR + i])

        rest = [pltpu.make_async_copy(s, d, sems.at[NR + 3 + i])
                for i, (s, d) in enumerate([(wg_hbm, wg_ref), (wu_hbm, wu_ref), (wd_hbm, wd_ref), (wo_hbm, wo_ref)])]

        def out_copy(r):
            return pltpu.make_async_copy(o_ref.at[pl.ds(r * FR, FR), :], out_hbm.at[pl.ds(r * FR, FR), :], sems.at[NR + 7 + r])

        x_copy(0).start()
        w_copy(1).start()
        for r in range(1, NR):
            x_copy(r).start()
        w_copy(0).start()
        w_copy(2).start()
        z_ref[0] = 0

        def layernorm(s):
            rows = pl.ds(s * SC, SC)
            x = x_ref[rows, :].astype(F32)
            mu = jnp.mean(x, axis=-1, keepdims=True)
            xc = x - mu
            var = jnp.mean(xc * xc, axis=-1, keepdims=True)
            xn_ref[rows, :] = (xc * jax.lax.rsqrt(var + 1e-5)).astype(BF16)

        def kproj(s):
            rows = pl.ds(s * SC, SC)
            kk = jnp.dot(xn_ref[rows, :], wqkv_ref[:, D:2 * D], preferred_element_type=F32)
            hi = jax.lax.broadcasted_iota(jnp.int32, (SC, 128), 1) >= 64
            for g in range(NG):
                k_ref[g, rows, :] = kk[:, g * 128:(g + 1) * 128].astype(BF16)
            for g in range(NG - 1):
                k_ref[NG + g, rows, :] = jnp.where(hi, kk[:, g * 128:(g + 1) * 128], kk[:, (g + 1) * 128:(g + 2) * 128]).astype(BF16)

        NSC = S // SC
        per = RC // SC
        x_copy(0).wait()
        layernorm(0)
        w_copy(1).wait()
        for s in range(1, NSC):
            if s % per == 0:
                x_copy(s // per).wait()
            if s == NSC - 1:
                w_copy(0).wait()
                w_copy(2).wait()
                for c in rest:
                    c.start()
            layernorm(s)
            kproj(s - 1)
        kproj(NSC - 1)
        wt_ref[0:D, :] = wqkv_ref[:, 0:D].astype(F32).T.astype(BF16)
        wt_ref[D:2 * D, :] = wqkv_ref[:, 2 * D:3 * D].astype(F32).T.astype(BF16)

        def qvproj(r, carry):
            rows = pl.ds(pl.multiple_of(r * RC, RC), RC)
            qvt = jax.lax.dot_general(wt_ref[...], xn_ref[rows, :], NT_DIMS, preferred_element_type=F32)
            for g in range(NG):
                q_ref[g, :, rows] = (qvt[g * 128:(g + 1) * 128, :] * QSCALE).astype(BF16)
            for g in range(NG - 1):
                q_ref[NG + g, 64:128, rows] = (qvt[g * 128 + 64:(g + 1) * 128, :] * QSCALE).astype(BF16)
                q_ref[NG + g, 0:64, rows] = (qvt[(g + 1) * 128:(g + 1) * 128 + 64, :] * QSCALE).astype(BF16)
            sub = jax.lax.broadcasted_iota(jnp.int32, (VR - DH, RC), 0)
            tail = jnp.where(sub == 0, 1.0, 0.0).astype(F32)
            for h in range(H):
                vt_ref[h, 0:DH, rows] = qvt[D + h * DH:D + (h + 1) * DH, :]
                vt_ref[h, DH:VR, rows] = tail
            return carry

        jax.lax.fori_loop(0, NR, qvproj, 0)

        def unit_idx(u):
            return u % H, u // H

        def qweights(u):
            h, j = unit_idx(u)
            lo = h * DH
            g0 = lo // 128
            g1 = (lo + DH - 1) // 128
            t = jnp.where(g0 == g1, g0, NG + g0)
            q = q_ref[t, :, pl.ds(pl.multiple_of(j * TQ, TQ), TQ)]
            idx = jax.lax.broadcasted_iota(jnp.int32, (128, TQ), 0)
            mask = ((idx - lo) & 127) < DH
            qm = jnp.where(mask, q.astype(F32), 0.0).astype(BF16)
            return t, qm

        def qk_chunk(t, qm, c, s_dst, mx):
            s = jnp.dot(k_ref[t, c * CK:(c + 1) * CK, :], qm, preferred_element_type=F32)
            s_dst[c * CK:(c + 1) * CK, :] = s
            part = jnp.max(s.reshape(CK // 8, 8, TQ), axis=0)
            return part if mx is None else jnp.maximum(mx, part)

        def run_stages(u0, n_stages, m, z, first_buf, last_has_qk=True):
            bufs = (sa_ref, sb_ref)
            pending = []
            state = {}

            def flush(n_keep):
                while len(pending) > n_keep:
                    k, c, p = pending.pop(0)
                    hc, jc = unit_idx(u0 + k)
                    d = jax.lax.dot_general(vt_ref[hc, :, c * CK:(c + 1) * CK], p, (((1,), (0,)), ((), ())), preferred_element_type=F32)
                    state[k] = d if c == 0 else state[k] + d
                    if c == NC - 1:
                        acc = state.pop(k)
                        ot_ref[hc, :, pl.ds(pl.multiple_of(jc * TQ, TQ), TQ)] = acc / acc[DH:DH + 1, :]

            for k in range(n_stages):
                src = bufs[(first_buf + k) % 2]
                dst = bufs[(first_buf + k + 1) % 2]
                has_qk = last_has_qk or k < n_stages - 1
                if has_qk:
                    t, qm = qweights(u0 + k + 1)
                mx = None
                for c in range(NC):
                    sv = src[pl.ds(pl.multiple_of(c * CK + z, CK), CK), :]
                    p = jnp.exp2(sv - m)
                    if PBF:
                        p = p.astype(BF16)
                    if has_qk:
                        mx = qk_chunk(t, qm, c, dst, mx)
                    pending.append((k, c, p))
                    flush(LAG)
                if has_qk:
                    m = jnp.max(mx, axis=0, keepdims=True)
            flush(0)
            return m

        t0, qm0 = qweights(0)
        mx0 = None
        for c in range(NC):
            mx0 = qk_chunk(t0, qm0, c, sa_ref, mx0)
        m0 = jnp.max(mx0, axis=0, keepdims=True)

        def att(i, m):
            return run_stages(NS * i, NS, m, z_ref[0], 0)

        m1 = jax.lax.fori_loop(0, n_iter, att, m0)
        for c in rest:
            c.wait()
        run_stages(NU - 2, 2, m1, z_ref[0], 0, last_has_qk=False)

        def final(r, carry):
            rows = pl.ds(pl.multiple_of(r * FR, FR), FR)
            xn = xn_ref[rows, :]
            ot = jnp.concatenate([ot_ref[h, 0:DH, rows] for h in range(H)], axis=0)
            o = ot.T.astype(BF16)
            attn = jnp.dot(o, wo_ref[...], preferred_element_type=F32)
            g = jnp.dot(xn, wg_ref[...], preferred_element_type=F32)
            u = jnp.dot(xn, wu_ref[...], preferred_element_type=F32)
            hmid = (g * jax.nn.sigmoid(g) * u).astype(BF16)
            y = jnp.dot(hmid, wd_ref[...], preferred_element_type=F32)
            o_ref[rows, :] = (x_ref[rows, :].astype(F32) + attn + y).astype(o_ref.dtype)
            pltpu.make_async_copy(o_ref.at[rows, :], out_hbm.at[rows, :], sems.at[NR + 7 + r]).start()
            return carry

        jax.lax.fori_loop(0, NFR, final, 0)
        for r in range(NFR):
            out_copy(r).wait()

    @jax.jit
    def f(A_x, A_wqkv, A_wo, B_x, B_w_gate, B_w_up, B_w_down):
        x = A_x.reshape(S, D)
        out = pl.pallas_call(
            kernel,
            out_shape=jax.ShapeDtypeStruct((S, D), BF16),
            in_specs=[pl.BlockSpec(memory_space=pl.ANY)] * 6,
            out_specs=pl.BlockSpec(memory_space=pl.ANY),
            scratch_shapes=[
                pltpu.VMEM((S, D), BF16),
                pltpu.VMEM((D, 3 * D), BF16),
                pltpu.VMEM((D, D), BF16),
                pltpu.VMEM((D, F), BF16),
                pltpu.VMEM((D, F), BF16),
                pltpu.VMEM((F, D), BF16),
                pltpu.VMEM((S, D), BF16),
                pltpu.VMEM((S, D), BF16),
                pltpu.VMEM((2 * NG - 1, 128, S), BF16),
                pltpu.VMEM((2 * NG - 1, S, 128), BF16),
                pltpu.VMEM((H, VR, S), F32),
                pltpu.VMEM((H, VR, S), F32),
                pltpu.VMEM((S, TQ), F32),
                pltpu.VMEM((S, TQ), F32),
                pltpu.VMEM((2 * D, D), BF16),
                pltpu.SMEM((1,), jnp.int32),
                pltpu.SemaphoreType.DMA((NR + 7 + NFR,)),
            ],
            compiler_params=pltpu.CompilerParams(vmem_limit_bytes=100 * 1024 * 1024),
        )(x, A_wqkv, A_wo, B_w_gate, B_w_up, B_w_down)
        return out.reshape(1, S, D)
    return f


pallas_parallel_sum__softmax_full_mha__swiglu_ffn__prompt_kernel = make_kernel()
```

```python
import math
import jax
import jax.numpy as jnp
import jax.experimental.pallas as pl
import jax.experimental.pallas.tpu as pltpu

S, D, F = 2048, 640, 1536
H, DH = 32, 20
VR = 24
NG = D // 128
NTILE = 2 * NG - 1
NT_DIMS = (((1,), (1,)), ((), ()))
NN_DIMS = (((1,), (0,)), ((), ()))
QSCALE = (DH ** -0.5) * math.log2(math.e)
F32 = jnp.float32
BF16 = jnp.bfloat16
SHIFT = 64.0
L_MIN = 2.0 ** -80
ACC_MAX = 2.0 ** 120


def head_tile(h):
    lo = h * DH
    g0, g1 = lo // 128, (lo + DH - 1) // 128
    return g0 if g0 == g1 else NG + g0


def _aux_rows():
    rows = {}
    for t in range(NTILE):
        heads = [h for h in range(H) if head_tile(h) == t]
        used = set((h * DH + d) % 128 for h in heads for d in range(DH))
        free = [r for r in range(128) if r not in used]
        assert len(free) >= len(heads)
        for h, r in zip(heads, free):
            rows[h] = r
    return [rows[h] for h in range(H)]


AUX = _aux_rows()


def make_kernel(TQ=512, CK=128, RC=512, LAG=1, FR=256, SC=128, NV=256, A=2, ATT=0, OFF=0, SPAN=100,
                GPOS=1, PF32=1, WK=2, FORCE=0):
    NQ = S // TQ
    NT = TQ // 128
    NC = S // CK
    NR = S // RC
    NFR = S // FR
    NM = S - NV
    assert RC == TQ and NV % (8 * A) == 0
    mb = [8 * ((NM // 8) * c // NC) for c in range(NC + 1)]
    items = [(kb, tb) for kb in range(NV // (8 * A)) for tb in range(NT)]
    WD = WK * 128
    WH = -(-WD // DH)

    def kernel(x_hbm, wqkv_hbm, wo_hbm, wg_hbm, wu_hbm, wd_hbm, out_hbm,
               x_ref, wqkv_ref, wo_ref, wg_ref, wu_ref, wd_ref, o_ref,
               xn_ref, q_ref, k_ref, vt_ref, ot_ref, wt_ref,
               kba_ref, kbb_ref, qf_ref, kn_ref, lm_ref, ap_ref, s_ref, sv_ref, aux_ref, sems):
        def x_copy(r):
            return pltpu.make_async_copy(x_hbm.at[pl.ds(r * RC, RC), :], x_ref.at[pl.ds(r * RC, RC), :], sems.at[r])

        def w_copy(i):
            return pltpu.make_async_copy(wqkv_hbm.at[:, pl.ds(i * D, D)], wqkv_ref.at[:, pl.ds(i * D, D)], sems.at[NR + i])

        rest = [pltpu.make_async_copy(s, d, sems.at[NR + 3 + i])
                for i, (s, d) in enumerate([(wo_hbm, wo_ref), (wg_hbm, wg_ref), (wu_hbm, wu_ref), (wd_hbm, wd_ref)])]

        def out_copy(r):
            return pltpu.make_async_copy(o_ref.at[pl.ds(r * FR, FR), :], out_hbm.at[pl.ds(r * FR, FR), :], sems.at[NR + 7 + r])

        x_copy(0).start()
        w_copy(1).start()
        for r in range(1, NR):
            x_copy(r).start()
        w_copy(0).start()
        w_copy(2).start()
        for h in range(H):
            aux_ref[h] = AUX[h]
        lm_ref[...] = jnp.full((8, TQ), ACC_MAX, F32)

        e_row = jax.lax.broadcasted_iota(jnp.int32, (H, D), 0)
        e_col = jax.lax.broadcasted_iota(jnp.int32, (H, D), 1)
        et = jnp.where((e_col >= e_row * DH) & (e_col < (e_row + 1) * DH), 1.0, 0.0).astype(BF16)

        def layernorm(s):
            rows = pl.ds(s * SC, SC)
            x = x_ref[rows, :].astype(F32)
            mu = jnp.mean(x, axis=-1, keepdims=True)
            xc = x - mu
            var = jnp.mean(xc * xc, axis=-1, keepdims=True)
            xn_ref[rows, :] = (xc * jax.lax.rsqrt(var + 1e-5)).astype(BF16)

        def kproj(s):
            rows = pl.ds(s * SC, SC)
            kk = jnp.dot(xn_ref[rows, :], wqkv_ref[:, D:2 * D], preferred_element_type=F32)
            kk = kk.astype(BF16).astype(F32)
            kn_ref[:, rows] = jax.lax.dot_general(et, (kk * kk).astype(BF16), NT_DIMS, preferred_element_type=F32)
            lane = jax.lax.broadcasted_iota(jnp.int32, (SC, 128), 1)
            tiles = [kk[:, g * 128:(g + 1) * 128] for g in range(NG)]
            tiles += [jnp.where(lane >= 64, tiles[g], tiles[g + 1]) for g in range(NG - 1)]
            for g, tl in enumerate(tiles):
                ar = [AUX[h] for h in range(H) if head_tile(h) == g]
                isaux = functools_reduce_or([lane == r for r in ar])
                k_ref[g, rows, :] = jnp.where(isaux, 1.0, tl)

        def functools_reduce_or(ms):
            out = ms[0]
            for m_ in ms[1:]:
                out = out | m_
            return out

        NSC = S // SC if not ATT else 1
        per = RC // SC
        x_copy(0).wait()
        layernorm(0)
        w_copy(1).wait()
        for s in range(1, NSC):
            if s % per == 0:
                x_copy(s // per).wait()
            if s == NSC - 1:
                w_copy(0).wait()
                w_copy(2).wait()
                for c in rest:
                    c.start()
            layernorm(s)
            kproj(s - 1)
        kproj(NSC - 1)
        if ATT:
            for r in range(1, NR):
                x_copy(r).wait()
            w_copy(0).wait()
            w_copy(2).wait()
            for c in rest:
                c.start()
        wt_ref[0:D, :] = wqkv_ref[:, 0:D].astype(F32).T.astype(BF16)
        wt_ref[D:2 * D, :] = wqkv_ref[:, 2 * D:3 * D].astype(F32).T.astype(BF16)
        kmax2 = jnp.max(kn_ref[...], axis=1, keepdims=True)

        def tile_of(h):
            lo = h * DH
            g0 = lo // 128
            g1 = (lo + DH - 1) // 128
            return jnp.where(g0 == g1, g0, NG + g0)

        def gen_kb(h, dst, d0, n):
            kv = k_ref[tile_of(h), NM:S, :]
            for i in range(n):
                ln = (h * DH + d0 + i) % 128
                dst[d0 + i] = jnp.take_along_axis(kv, jnp.full((NV, 128), ln, jnp.int32), axis=1)

        def qweights(h, cols, with_aux=True):
            q = q_ref[tile_of(h), :, cols]
            idx = jax.lax.broadcasted_iota(jnp.int32, (128, TQ), 0)
            mask = ((idx - h * DH) & 127) < DH
            if with_aux:
                mask = mask | (idx == aux_ref[h])
            return jnp.where(mask, q.astype(F32), 0.0).astype(BF16)

        def qvproj(r, carry):
            rows = pl.ds(pl.multiple_of(r * RC, RC), RC)
            xn = xn_ref[rows, :]
            qt = jax.lax.dot_general(wt_ref[0:D, :], xn, NT_DIMS, preferred_element_type=F32)
            qf = (qt * QSCALE).astype(BF16).astype(F32)
            qn2 = jnp.dot(et, (qf * qf).astype(BF16), preferred_element_type=F32)
            vt = jax.lax.dot_general(wt_ref[D:2 * D, :], xn, NT_DIMS, preferred_element_type=F32)
            negm = (SHIFT - jnp.sqrt(qn2 * kmax2)).astype(BF16).astype(F32)
            idx = jax.lax.broadcasted_iota(jnp.int32, (16, RC), 0)
            for g in range(NTILE):
                if g < NG:
                    tl = qf[g * 128:(g + 1) * 128, :]
                else:
                    g0 = g - NG
                    tl = jnp.concatenate([qf[(g0 + 1) * 128:(g0 + 1) * 128 + 64, :], qf[g0 * 128 + 64:(g0 + 1) * 128, :]], axis=0)
                for b in range(8):
                    blk = tl[b * 16:(b + 1) * 16, :]
                    for h in range(H):
                        if head_tile(h) == g and AUX[h] // 16 == b:
                            blk = jnp.where(idx == AUX[h] % 16, negm[h:h + 1, :], blk)
                    q_ref[g, b * 16:(b + 1) * 16, rows] = blk.astype(BF16)
            for h in range(H):
                for t in range(RC // 128):
                    qf_ref[h, r * (RC // 128) + t, 0:DH, :] = qf[h * DH:(h + 1) * DH, t * 128:(t + 1) * 128]
                    qf_ref[h, r * (RC // 128) + t, DH:DH + 1, :] = negm[h:h + 1, t * 128:(t + 1) * 128]
            sub = jax.lax.broadcasted_iota(jnp.int32, (VR - DH, RC), 0)
            tail = jnp.where(sub == 0, 1.0, 0.0).astype(F32)
            for h in range(H):
                vt_ref[h, 0:DH, rows] = vt[h * DH:(h + 1) * DH, :]
                vt_ref[h, DH:VR, rows] = tail
            qm = qweights(0, rows)
            s_ref[r] = jax.lax.dot_general(k_ref[0, 0:NM, :], qm, NN_DIMS, preferred_element_type=F32)
            sv_ref[r] = jax.lax.dot_general(k_ref[0, NM:S, :], qm, NN_DIMS, preferred_element_type=F32)
            gen_kb(1, kbb_ref, r * (DH // NR), DH // NR)
            return carry

        if not ATT:
            jax.lax.fori_loop(0, NR, qvproj, 0)

        def finish_unit(h, cols, acc):
            l = acc[DH:DH + 1, :]
            big = jnp.max(jnp.abs(acc), axis=0, keepdims=True)
            lm_ref[...] = jnp.minimum(lm_ref[...], jnp.where(big < ACC_MAX, l, 0.0))
            ot_ref[h, :, cols] = acc / l

        def head_body(par, hq, hs, filler=None):
            kb_src = (kba_ref, kbb_ref)[par]
            kb_dst = (kbb_ref, kba_ref)[par]
            pending = []
            state = {}

            def flush(n_keep):
                while len(pending) > n_keep:
                    js, c, p = pending.pop(0)
                    d = jax.lax.dot_general(vt_ref[hs, :, c * CK:(c + 1) * CK], p, NN_DIMS, preferred_element_type=F32)
                    state[js] = d if c == 0 else state[js] + d
                    if c == NC - 1:
                        finish_unit(hs, slice(js * TQ, (js + 1) * TQ), state.pop(js))

            for j in range(NQ):
                js = (j + 1) % NQ
                src = s_ref.at[js if js else NQ * (1 - par)]
                dst = s_ref.at[j if j else NQ * par]
                vsrc = sv_ref.at[(1 - par) * NQ + js]
                vdst = sv_ref.at[par * NQ + j]
                if hq is not None:
                    t = tile_of(hq)
                    qm = qweights(hq, slice(j * TQ, (j + 1) * TQ))
                done = 0

                def vpu_item(kb_i, tt):
                    def rep(v):
                        return jnp.concatenate([v] * A, axis=0) if A > 1 else v
                    acc = rep(qf_ref[hq, j * NT + tt, pl.ds(DH, 8, stride=0), :])
                    for d in range(DH):
                        kb = kb_src[d, kb_i * 8 * A:(kb_i + 1) * 8 * A, :]
                        acc = acc + kb * rep(qf_ref[hq, j * NT + tt, pl.ds(d, 8, stride=0), :])
                    vdst[kb_i * 8 * A:(kb_i + 1) * 8 * A, tt * 128:(tt + 1) * 128] = acc
                    pin = acc if A == 1 else jnp.max(acc.reshape(A, 8, 128), axis=0)
                    return pin - pin

                pos = [OFF + ((i + 1) * (NM * SPAN // 100 - OFF)) // len(items) // 8 * 8 - 8 for i in range(len(items))]
                for c in range(NC):
                    lo_r, hi_r = c * CK, (c + 1) * CK
                    parts = []
                    if lo_r < NM:
                        parts.append(src[lo_r:min(hi_r, NM), :])
                    if hi_r > NM:
                        parts.append(vsrc[max(lo_r, NM) - NM:hi_r - NM, :])
                    sv = parts[0] if len(parts) == 1 else jnp.concatenate(parts, axis=0)
                    p = jnp.exp2(sv)
                    if not PF32:
                        p = p.astype(BF16)
                    if hq is not None:
                        kc = k_ref[t, mb[c]:mb[c + 1], :]
                        n = mb[c + 1] - mb[c]
                        if done < len(items) and pos[done] < mb[c + 1]:
                            groups = [kc[r:r + 8, :] for r in range(0, n, 8)]
                            while done < len(items) and pos[done] < mb[c + 1]:
                                z0 = vpu_item(*items[done])
                                gi = (pos[done] - mb[c]) // 8
                                groups[gi] = groups[gi] + z0
                                done += 1
                            kc = jnp.concatenate(groups, axis=0)
                        dst[mb[c]:mb[c + 1], :] = jax.lax.dot_general(kc, qm, NN_DIMS, preferred_element_type=F32)
                    if filler is not None:
                        filler(j * NC + c)
                    pending.append((js, c, p))
                    flush(LAG)
                    if hq is not None and c == GPOS:
                        gen_kb(jnp.minimum(hq + 1, H - 1), kb_dst, j * (DH // NQ), DH // NQ)
            flush(0)

        def att(i, carry):
            @pl.when(i % 2 == 0)
            def _():
                head_body(0, i, i - 1)

            @pl.when(i % 2 == 1)
            def _():
                head_body(1, i, i - 1)
            return carry

        jax.lax.fori_loop(1, H, att, 0)
        for c in rest:
            c.wait()

        def wo_partial(rows):
            ot = jnp.concatenate([ot_ref[h, 0:DH, rows] for h in range(WH)], axis=0)[0:WD, :]
            ap_ref[rows, :] = jnp.dot(ot.T.astype(BF16), wo_ref[0:WD, :], preferred_element_type=F32)

        PB = 128
        every = (NQ * NC) // (S // PB)

        def filler(step):
            if step % every == 0:
                b = step // every
                wo_partial(slice(b * PB, (b + 1) * PB))

        head_body(H % 2, None, H - 1, filler=filler)

        lmin = jnp.min(lm_ref[...])
        unsafe = jnp.logical_not(lmin >= L_MIN)
        if FORCE:
            unsafe = lmin >= -1.0

        @pl.when(unsafe)
        def _():
            FK = 256

            def exact_unit(u, carry):
                h = u // NQ
                cols = pl.ds(pl.multiple_of((u % NQ) * TQ, TQ), TQ)
                t = tile_of(h)
                qm = qweights(h, cols, with_aux=False)

                def chunk(c, st):
                    m, acc = st
                    rows = pl.ds(pl.multiple_of(c * FK, FK), FK)
                    s = jax.lax.dot_general(k_ref[t, rows, :], qm, NN_DIMS, preferred_element_type=F32)
                    m_new = jnp.maximum(m, jnp.max(s, axis=0, keepdims=True))
                    p = jnp.exp2(s - m_new)
                    acc = acc * jnp.exp2(m - m_new) + jnp.dot(vt_ref[h, :, rows], p, preferred_element_type=F32)
                    return m_new, acc

                s0 = jax.lax.dot_general(k_ref[t, 0:8, :], qm, NN_DIMS, preferred_element_type=F32)
                m0 = jnp.max(s0, axis=0, keepdims=True)
                _, acc = jax.lax.fori_loop(0, S // FK, chunk, (m0, jnp.zeros((VR, TQ), F32)))
                ot_ref[h, :, cols] = acc / acc[DH:DH + 1, :]
                return carry

            jax.lax.fori_loop(0, H * NQ, exact_unit, 0)

            def redo(b, carry):
                wo_partial(pl.ds(pl.multiple_of(b * PB, PB), PB))
                return carry

            jax.lax.fori_loop(0, S // PB, redo, 0)

        def final(r, carry):
            rows = pl.ds(pl.multiple_of(r * FR, FR), FR)
            xn = xn_ref[rows, :]
            h0 = WD // DH
            ot = jnp.concatenate([ot_ref[h, 0:DH, rows] for h in range(h0, H)], axis=0)[WD - h0 * DH:, :]
            o = ot.T.astype(BF16)
            if ATT:
                o_ref[rows, 0:D - WD] = o
            else:
                g = jnp.dot(xn, wg_ref[...], preferred_element_type=F32)
                u = jnp.dot(xn, wu_ref[...], preferred_element_type=F32)
                attn = jnp.dot(o, wo_ref[WD:D, :], preferred_element_type=F32)
                hmid = (g * jax.nn.sigmoid(g) * u).astype(BF16)
                y = jnp.dot(hmid, wd_ref[...], preferred_element_type=F32)
                o_ref[rows, :] = (x_ref[rows, :].astype(F32) + ap_ref[rows, :] + attn + y).astype(o_ref.dtype)
            pltpu.make_async_copy(o_ref.at[rows, :], out_hbm.at[rows, :], sems.at[NR + 7 + r]).start()
            return carry

        jax.lax.fori_loop(0, NFR, final, 0)
        for r in range(NFR):
            out_copy(r).wait()

    @jax.jit
    def f(A_x, A_wqkv, A_wo, B_x, B_w_gate, B_w_up, B_w_down):
        x = A_x.reshape(S, D)
        out = pl.pallas_call(
            kernel,
            out_shape=jax.ShapeDtypeStruct((S, D), BF16),
            in_specs=[pl.BlockSpec(memory_space=pl.ANY)] * 6,
            out_specs=pl.BlockSpec(memory_space=pl.ANY),
            scratch_shapes=[
                pltpu.VMEM((S, D), BF16),
                pltpu.VMEM((D, 3 * D), BF16),
                pltpu.VMEM((D, D), BF16),
                pltpu.VMEM((D, F), BF16),
                pltpu.VMEM((D, F), BF16),
                pltpu.VMEM((F, D), BF16),
                pltpu.VMEM((S, D), BF16),
                pltpu.VMEM((S, D), BF16),
                pltpu.VMEM((NTILE, 128, S), BF16),
                pltpu.VMEM((NTILE, S, 128), F32),
                pltpu.VMEM((H, VR, S), F32),
                pltpu.VMEM((H, VR, S), F32),
                pltpu.VMEM((2 * D, D), BF16),
                pltpu.VMEM((DH, NV, 128), F32),
                pltpu.VMEM((DH, NV, 128), F32),
                pltpu.VMEM((H, S // 128, VR, 128), F32),
                pltpu.VMEM((H, S), F32),
                pltpu.VMEM((8, TQ), F32),
                pltpu.VMEM((S, D), F32),
                pltpu.VMEM((NQ + 1, NM, TQ), F32),
                pltpu.VMEM((2 * NQ, NV, TQ), F32),
                pltpu.SMEM((H,), jnp.int32),
                pltpu.SemaphoreType.DMA((NR + 7 + NFR,)),
            ],
            compiler_params=pltpu.CompilerParams(vmem_limit_bytes=120 * 1024 * 1024),
        )(x, A_wqkv, A_wo, B_w_gate, B_w_up, B_w_down)
        return out.reshape(1, S, D)
    return f


pallas_parallel_sum__softmax_full_mha__swiglu_ffn__prompt_kernel = make_kernel()
```

```python
import math

import jax
import jax.numpy as jnp
import jax.experimental.pallas as pl
import jax.experimental.pallas.tpu as pltpu

S, D, F = 2048, 640, 1536
H, DH = 32, 20
VR = 24
QR = 32
NG = D // 128
NTILE = 2 * NG - 1
NT_DIMS = (((1,), (1,)), ((), ()))
NN_DIMS = (((1,), (0,)), ((), ()))
QSCALE = (DH ** -0.5) * math.log2(math.e)
F32 = jnp.float32
BF16 = jnp.bfloat16

SHIFT = 64.0
L_MIN = 2.0 ** -80
L_MAX = 2.0 ** 80
V_MAX = 2.0 ** 40

TQ = 512
CK = 128
SC = 128
FR = 256
PB = 128
FK = 128
NV = 384
KB_PAD = 8
HG = 768
UR = 128
NFUSE = F // HG
VA = 2
WD = 256
VS = 480
XB = [0, 3, 9, 16]
XW = {2: [1], 8: [2]}
WAIT_B, T_POS = 8, 9
NX = len(XB) - 1
PIN_OFF, N_FREE, PIN_FRAC, PIN_TIME = 32, 3, 0.75, 0.72
DENSE_FIRST, DENSE_LAST, ACT_DELAY, N_EARLY = 1, 60, 2, 48

NQ = S // TQ
NT = TQ // 128
NC = S // CK
NFR = S // FR
NM = S - NV
KQ = -(-NM // (8 * NQ)) * 8
ROW_BOUNDS = [8 * ((NM // 8) * c // NC) for c in range(NC + 1)]
ITEMS = [(ju, kb, tt) for ju in range(NQ) for tt in range(NT) for kb in range(NV // (8 * VA))]


def _head_tile(h):
    lo = h * DH
    g0, g1 = lo // 128, (lo + DH - 1) // 128
    return g0 if g0 == g1 else NG + g0


NH = HG // 128


def _out_pieces(nk):
    out = []
    k0 = 0
    while nk - k0 >= 4:
        out += [(k0, k0 + 4, n, n + 1) for n in range(NG)]
        k0 += 4
    rem = nk - k0
    if rem:
        step = 4 // rem
        out += [(k0, nk, n, min(n + step, NG)) for n in range(0, NG, step)]
    return out


K4 = [("k4", i) for i in range(0, 2 * NH, 4)]
GU = [("gu", i) for i in range(2 * NH)]
DOWN = [("down", b) for b in _out_pieces(NH)]
DENSE = K4 + GU + DOWN


def _piece_time(p):
    kind, a = p
    if kind == "k4":
        return UR * min(4, 2 * NH - a) // 4
    if kind == "gu":
        return UR
    return UR * (a[1] - a[0]) * (a[3] - a[2]) // 4


DENSE_AT = {}
_first, _last = DENSE_FIRST, DENSE_LAST
for _p in range(len(DENSE)):
    DENSE_AT.setdefault(_first + (_p * (_last - _first)) // (len(DENSE) - 1), []).append(DENSE[_p])


def _pin_positions():
    n = len(ITEMS) - N_FREE
    total = NQ * NM + NQ * NC * VR + sum(_piece_time(p) for p in DENSE) - PIN_OFF
    pos = []
    for i in range(n):
        fr = (i + 1) / n
        if fr <= PIN_FRAC:
            t = fr / PIN_FRAC * PIN_TIME
        else:
            t = PIN_TIME + (fr - PIN_FRAC) / (1 - PIN_FRAC) * (1 - PIN_TIME)
        pos.append(max(0, (PIN_OFF + int(t * total)) // 8 * 8 - 8))
    return pos


PIN_POS = _pin_positions()


def _kernel(x_hbm, wqkv_hbm, wo_hbm, wg_hbm, wu_hbm, wd_hbm, out_hbm,
            x_ref, wqkv_ref, wo_ref, wg_ref, wu_ref, wd_ref, o_ref,
            xn_ref, qc_ref, k_ref, vt_ref, ot_ref, wt_ref,
            kba_ref, kbb_ref, kra_ref, krb_ref, qf_ref, kn_ref, lm_ref, ap_ref,
            s_ref, sv_ref, xf_ref, ha_ref, hb_ref, aw_ref, tile_ref, sems):
    def x_copy(r):
        rows = pl.ds(XB[r] * SC, (XB[r + 1] - XB[r]) * SC)
        return pltpu.make_async_copy(x_hbm.at[rows, :], x_ref.at[rows, :], sems.at[r])

    def w_copy(i):
        cols = pl.ds(i * D, D)
        return pltpu.make_async_copy(wqkv_hbm.at[:, cols], wqkv_ref.at[:, cols], sems.at[NX + i])

    late = [pltpu.make_async_copy(src, dst, sems.at[NX + 3 + i])
            for i, (src, dst) in enumerate([(wo_hbm, wo_ref), (wg_hbm, wg_ref), (wu_hbm, wu_ref), (wd_hbm, wd_ref)])]

    def out_copy(rows, r):
        return pltpu.make_async_copy(o_ref.at[rows, :], out_hbm.at[rows, :], sems.at[NX + 7 + r])

    x_copy(0).start()
    w_copy(1).start()
    for r in range(1, NX):
        x_copy(r).start()
    w_copy(0).start()
    w_copy(2).start()
    for h in range(H):
        tile_ref[h] = _head_tile(h)
    for a in range(VA):
        tile_ref[H + a] = 128 + a
    lm_ref[0] = jnp.full((8, TQ), 1.0, F32)
    lm_ref[1] = jnp.full((8, TQ), 1.0, F32)
    lm_ref[2] = jnp.zeros((8, TQ), F32)

    e_row = jax.lax.broadcasted_iota(jnp.int32, (H, D), 0)
    e_col = jax.lax.broadcasted_iota(jnp.int32, (H, D), 1)
    head_sel = jnp.where((e_col >= e_row * DH) & (e_col < (e_row + 1) * DH), 1.0, 0.0).astype(BF16)

    def layernorm(s):
        rows = pl.ds(s * SC, SC)
        x = x_ref[rows, :].astype(F32)
        mu = jnp.mean(x, axis=-1, keepdims=True)
        xc = x - mu
        var = jnp.mean(xc * xc, axis=-1, keepdims=True)
        xn = (xc * jax.lax.rsqrt(var + 1e-5)).astype(BF16)
        xn_ref[rows, :] = xn
        xf_ref[rows, :] = xn.astype(F32)

    def knorm(s, kk2):
        kn_ref[:, pl.ds(s * SC, SC)] = jax.lax.dot_general(head_sel, kk2, NT_DIMS, preferred_element_type=F32)

    def kproj(s):
        rows = pl.ds(s * SC, SC)
        kk = jnp.dot(xn_ref[rows, :], wqkv_ref[:, D:2 * D], preferred_element_type=F32)
        kk = kk.astype(BF16).astype(F32)
        lane = jax.lax.broadcasted_iota(jnp.int32, (SC, 128), 1)
        tiles = [kk[:, g * 128:(g + 1) * 128] for g in range(NG)]
        tiles += [jnp.where(lane >= 64, tiles[g], tiles[g + 1]) for g in range(NG - 1)]
        for g, tl in enumerate(tiles):
            k_ref[g, rows, :] = tl
        return (kk * kk).astype(BF16)

    n_sub = S // SC
    per = XB[1]
    x_copy(0).wait()
    for s in range(per):
        layernorm(s)
    w_copy(1).wait()
    prev = None
    for s in range(n_sub):
        for r in XW.get(s, []):
            x_copy(r).wait()
        if s == WAIT_B:
            w_copy(0).wait()
            w_copy(2).wait()
            for c in late:
                c.start()
        if per <= s + 1 < n_sub:
            layernorm(s + 1)
        if s == T_POS:
            wt_ref[0:D, :] = wqkv_ref[:, 0:D].astype(F32).T.astype(BF16)
            wt_ref[D:2 * D, :] = wqkv_ref[:, 2 * D:3 * D].astype(F32).T.astype(BF16)
        kk2 = kproj(s)
        if prev is not None:
            knorm(s - 1, prev)
        prev = kk2
    knorm(n_sub - 1, prev)
    kmax2 = jnp.max(kn_ref[...], axis=1, keepdims=True)

    def gen_kb(h, dst, d0, n):
        kv = k_ref[tile_ref[h], NM:S, :]
        for i in range(n):
            ln = (h * DH + d0 + i) % 128
            dst[d0 + i, 0:NV, :] = jnp.take_along_axis(kv, jnp.full((NV, 128), ln, jnp.int32), axis=1)

    def rotated_k(h, rows, n):
        kr = pltpu.roll(k_ref[tile_ref[h], rows, :], (D - h * DH) % 128, 1)
        lane = jax.lax.broadcasted_iota(jnp.int32, (n, 128), 1)
        return jnp.where(lane == DH, 1.0, kr)

    def scores(kc, qc):
        qm = jnp.concatenate([qc, jnp.zeros((128 - QR, TQ), BF16)], axis=0)
        return jax.lax.dot_general(kc, qm, NN_DIMS, preferred_element_type=F32)

    def qvproj(r, carry):
        rows = pl.ds(pl.multiple_of(r * TQ, TQ), TQ)
        xn = xn_ref[rows, :]
        qt = jax.lax.dot_general(wt_ref[0:D, :], xn, NT_DIMS, preferred_element_type=F32)
        qf = (qt * QSCALE).astype(BF16).astype(F32)
        vt0 = jax.lax.dot_general(wt_ref[D:D + VS, :], xn, NT_DIMS, preferred_element_type=F32)
        qn2 = jnp.dot(head_sel, (qf * qf).astype(BF16), preferred_element_type=F32)
        vt1 = jax.lax.dot_general(wt_ref[D + VS:2 * D, :], xn, NT_DIMS, preferred_element_type=F32)
        vt = jnp.concatenate([vt0, vt1], axis=0)
        lm_ref[2] = jnp.maximum(lm_ref[2], jnp.max(jnp.abs(vt).reshape(D // 8, 8, TQ), axis=0))
        negm = (SHIFT - jnp.sqrt(qn2 * kmax2)).astype(BF16).astype(F32)
        sub = jax.lax.broadcasted_iota(jnp.int32, (VR - DH, TQ), 0)
        tail = jnp.where(sub == 0, 1.0, 0.0).astype(F32)
        zpad = jnp.zeros((QR - VR, TQ), F32)
        for h in range(H):
            blk = jnp.concatenate([qf[h * DH:(h + 1) * DH, :], tail * negm[h:h + 1, :]], axis=0)
            qf_ref[h, :, rows] = blk
            qc_ref[h, :, rows] = jnp.concatenate([blk, zpad], axis=0).astype(BF16)
            vt_ref[h, 0:DH, rows] = vt[h * DH:(h + 1) * DH, :]
            vt_ref[h, DH:VR, rows] = tail
        lane = jax.lax.broadcasted_iota(jnp.int32, (S, 128), 1)
        s0 = scores(jnp.where(lane == DH, 1.0, k_ref[0]), qc_ref[0, :, rows])
        s_ref[r] = s0[0:NM]
        sv_ref[r] = s0[NM:S]
        gen_kb(1, kbb_ref, r * (DH // NQ), DH // NQ)
        krows = pl.ds(pl.multiple_of(r * KQ, 8), KQ)
        krb_ref[krows, :] = rotated_k(1, krows, KQ)
        return carry

    jax.lax.fori_loop(0, NQ, qvproj, 0)

    def activation(g, u):
        hg = 0.5 * g
        return (hg * (1.0 + jnp.tanh(hg))) * u

    def head_body(par, hq, hs, filler=None):
        kb_src, kb_dst = ((kba_ref, kbb_ref), (kbb_ref, kba_ref))[par]
        kr_src, kr_dst = ((kra_ref, krb_ref), (krb_ref, kra_ref))[par]
        h_dst, h_src = ((ha_ref, hb_ref), (hb_ref, ha_ref))[par]
        lane8 = jax.lax.broadcasted_iota(jnp.int32, (8, 128), 1)
        keep = [lane8 < tile_ref[H + a] for a in range(VA)]
        qrows = {}
        st = dict(done=0, t=0)

        def q_rows(tile):
            if tile not in qrows:
                blk = qf_ref[hq, :, tile * 128:(tile + 1) * 128]
                qrows[tile] = [jnp.concatenate([jnp.broadcast_to(blk[i:i + 1, :], (8, 128))] * VA, axis=0)
                               for i in range(DH + 1)]
            return qrows[tile]

        def vpu_item(ju, kb_i, tt):
            keys = slice(kb_i * 8 * VA, (kb_i + 1) * 8 * VA)
            q = q_rows(ju * NT + tt)
            acc = q[DH]
            for d in range(DH):
                acc = acc + kb_src[d, keys, :] * q[d]
            sv_ref[par * NQ + ju, keys, tt * 128:(tt + 1) * 128] = acc
            return acc

        def pinned(lhs, dur=None):
            n = lhs.shape[0]
            dur = n if dur is None else dur
            groups = [lhs[r:r + 8, :] for r in range(0, n, 8)]
            while st["done"] < len(PIN_POS) and PIN_POS[st["done"]] < st["t"] + dur:
                res = vpu_item(*ITEMS[st["done"]])
                gi = (PIN_POS[st["done"]] - st["t"]) // 8
                g0 = groups[gi][:, 0:128]
                for a in range(VA):
                    g0 = jnp.where(keep[a], g0, res[a * 8:(a + 1) * 8])
                groups[gi] = g0 if lhs.shape[1] == 128 else jnp.concatenate([g0, groups[gi][:, 128:]], axis=1)
                st["done"] += 1
            st["t"] += dur
            return jnp.concatenate(groups, axis=0)

        acts = []
        k4 = {}

        def wtile(i, k0, k1):
            n, w = divmod(i, 2)
            return (wg_ref, wu_ref)[w][k0:k1, par * HG + n * 128:par * HG + (n + 1) * 128]

        def dense(p):
            kind, a = p
            rows = pl.ds(pl.multiple_of((hq // NFUSE) * UR, UR), UR)
            if kind == "k4":
                ids = list(range(a, min(a + 4, 2 * NH)))
                lhs = pinned(xf_ref[rows, 512:640], _piece_time(p))
                w = jnp.concatenate([wtile(i, 512, 640) for i in ids], axis=1)
                res = jax.lax.dot_general(lhs, w, NN_DIMS, preferred_element_type=F32)
                for o, i in enumerate(ids):
                    k4[i] = res[:, o * 128:(o + 1) * 128]
            elif kind == "gu":
                lhs = pinned(xf_ref[rows, 0:512])
                k4[a] = jax.lax.dot_general(lhs, wtile(a, 0, 512), NN_DIMS, preferred_element_type=F32) + k4[a]
                if a % 2 == 1:
                    acts.append([ACT_DELAY, a // 2, k4[a - 1], k4[a]])
            else:
                down_piece(hs, 1 - par, a, pinned(h_src[:, a[0] * 128:a[1] * 128], _piece_time(p)))

        def tick():
            for a in list(acts):
                a[0] -= 1
                if a[0] <= 0:
                    h_dst[:, a[1] * 128:(a[1] + 1) * 128] = activation(a[2], a[3])
                    acts.pop(0)

        for j in range(NQ):
            js = (j + 1) % NQ
            src = s_ref.at[js if js else NQ * (1 - par)]
            dst = s_ref.at[j if j else NQ * par]
            vsrc = sv_ref.at[(1 - par) * NQ + js]
            if hq is not None:
                qc = qc_ref[hq, :, j * TQ:(j + 1) * TQ]
            acc_o = None
            for c in range(NC):
                lo, hi = c * CK, (c + 1) * CK
                parts = []
                if lo < NM:
                    parts.append(src[lo:min(hi, NM), :])
                if hi > NM:
                    parts.append(vsrc[max(lo, NM) - NM:hi - NM, :])
                sv = parts[0] if len(parts) == 1 else jnp.concatenate(parts, axis=0)
                vl = vt_ref[hs, :, lo:hi]
                pv = jnp.dot(pinned(vl) if hq is not None else vl, jnp.exp2(sv), preferred_element_type=F32)
                acc_o = pv if c == 0 else acc_o + pv
                if c == NC - 1:
                    lrows = acc_o[VR - 8:VR, :]
                    lm_ref[0] = jnp.minimum(lm_ref[0], lrows)
                    lm_ref[1] = jnp.maximum(lm_ref[1], lrows)
                    ot_ref[hs, :, js * TQ:(js + 1) * TQ] = acc_o
                if hq is not None:
                    r0, r1 = ROW_BOUNDS[c], ROW_BOUNDS[c + 1]
                    dst[r0:r1, :] = scores(pinned(kr_src[r0:r1, :]), qc)
                    tick()
                    for p in DENSE_AT.get(j * NC + c, []):
                        dense(p)
                    if c == 1:
                        hn = jnp.minimum(hq + 1, H - 1)
                        gen_kb(hn, kb_dst, j * (DH // NQ), DH // NQ)
                        kr_dst[j * KQ:(j + 1) * KQ, :] = rotated_k(hn, slice(j * KQ, (j + 1) * KQ), KQ)
                if filler is not None:
                    filler(j * NC + c)
        if hq is not None:
            assert not acts
            for it in ITEMS[st["done"]:]:
                vpu_item(*it)

    def down_piece(u, g, blk, hval):
        k0, k1, n0, n1 = blk
        if isinstance(u, int):
            rows = slice((u // NFUSE) * UR, (u // NFUSE + 1) * UR)
        else:
            rows = pl.ds(pl.multiple_of((u // NFUSE) * UR, UR), UR)
        cols = slice(n0 * 128, n1 * 128)
        y = jax.lax.dot_general(hval, wd_ref[g * HG + k0 * 128:g * HG + k1 * 128, cols], NN_DIMS,
                                preferred_element_type=F32)
        ap_ref[rows, cols] = y if (g == 0 and k0 == 0) else ap_ref[rows, cols] + y

    for c in late:
        c.wait()
    xn0 = xn_ref[0:UR, :]
    ha_ref[...] = activation(jnp.dot(xn0, wg_ref[:, 0:HG], preferred_element_type=F32),
                             jnp.dot(xn0, wu_ref[:, 0:HG], preferred_element_type=F32))

    def att(i, carry):
        @pl.when(i % 2 == 0)
        def _():
            head_body(0, i, i - 1)

        @pl.when(i % 2 == 1)
        def _():
            head_body(1, i, i - 1)
        return carry

    jax.lax.fori_loop(1, H, att, 0)

    def normalized(h, rows):
        return ot_ref[h, 0:DH, rows] / ot_ref[h, DH:DH + 1, rows]

    def wo_lhs(rows):
        ot = jnp.concatenate([normalized(h, rows) for h in range(-(-WD // DH))], axis=0)[0:WD, :]
        return ot.T.astype(BF16)

    lhs_cache = {}
    jobs = [("down", blk) for _, blk in DOWN] + [(b, blk) for b in range(S // PB) for blk in _out_pieces(WD // 128)]
    n_early = N_EARLY

    def run_job(job):
        b, blk = job
        k0, k1, n0, n1 = blk
        if b == "down":
            down_piece(H - 1, (H - 1) % 2, blk, hb_ref[:, k0 * 128:k1 * 128])
            return
        rows = slice(b * PB, (b + 1) * PB)
        if b not in lhs_cache:
            lhs_cache[b] = wo_lhs(rows)
        assert k0 == 0 and k1 * 128 == WD
        aw_ref[rows, n0 * 128:n1 * 128] = jnp.dot(lhs_cache[b], wo_ref[0:WD, n0 * 128:n1 * 128],
                                                  preferred_element_type=F32)

    def filler(k):
        for i in range(k * n_early // (NQ * NC), (k + 1) * n_early // (NQ * NC)):
            run_job(jobs[i])

    head_body(H % 2, None, H - 1, filler=filler)
    for job in jobs[n_early:]:
        run_job(job)

    lr = DH - (VR - 8)
    safe = ((jnp.min(lm_ref[0, lr:lr + 1, :]) >= L_MIN) & (jnp.max(lm_ref[1, lr:lr + 1, :]) <= L_MAX)
            & (jnp.max(lm_ref[2]) <= V_MAX))

    @pl.when(jnp.logical_not(safe))
    def _():
        def exact_unit(u, carry):
            h = u // NQ
            cols = pl.ds(pl.multiple_of((u % NQ) * TQ, TQ), TQ)
            idx = jax.lax.broadcasted_iota(jnp.int32, (QR, TQ), 0)
            qc = jnp.where(idx < DH, qc_ref[h, :, cols].astype(F32), 0.0).astype(BF16)

            def chunk(c, st):
                m, acc = st
                rows = pl.ds(pl.multiple_of(c * FK, FK), FK)
                s = scores(rotated_k(h, rows, FK), qc)
                m_new = jnp.maximum(m, jnp.max(s, axis=0, keepdims=True))
                p = jnp.exp2(s - m_new)
                acc = acc * jnp.exp2(m - m_new) + jnp.dot(vt_ref[h, :, rows], p, preferred_element_type=F32)
                return m_new, acc

            m0 = jnp.max(scores(rotated_k(h, slice(0, 8), 8), qc), axis=0, keepdims=True)
            _, acc = jax.lax.fori_loop(0, S // FK, chunk, (m0, jnp.zeros((VR, TQ), F32)))
            ot_ref[h, :, cols] = acc
            return carry

        jax.lax.fori_loop(0, H * NQ, exact_unit, 0)

        def redo(b, carry):
            rows = pl.ds(pl.multiple_of(b * PB, PB), PB)
            aw_ref[rows, :] = jnp.dot(wo_lhs(rows), wo_ref[0:WD, :], preferred_element_type=F32)
            return carry

        jax.lax.fori_loop(0, S // PB, redo, 0)

    h0 = WD // DH
    for r in range(NFR):
        rows = pl.ds(r * FR, FR)
        ot = jnp.concatenate([normalized(h, rows) for h in range(h0, H)], axis=0)[WD - h0 * DH:, :]
        acc = x_ref[rows, :].astype(F32) + ap_ref[rows, :] + aw_ref[rows, :]
        attn = jnp.dot(ot.T.astype(BF16), wo_ref[WD:D, :], preferred_element_type=F32)
        o_ref[rows, :] = (acc + attn).astype(o_ref.dtype)
        out_copy(rows, r).start()
    for r in range(NFR):
        out_copy(pl.ds(r * FR, FR), r).wait()


@jax.jit
def pallas_parallel_sum__softmax_full_mha__swiglu_ffn__prompt_kernel(
    A_x: jax.Array,
    A_wqkv: jax.Array,
    A_wo: jax.Array,
    B_x: jax.Array,
    B_w_gate: jax.Array,
    B_w_up: jax.Array,
    B_w_down: jax.Array,
):
    out = pl.pallas_call(
        _kernel,
        out_shape=jax.ShapeDtypeStruct((S, D), BF16),
        in_specs=[pl.BlockSpec(memory_space=pl.ANY)] * 6,
        out_specs=pl.BlockSpec(memory_space=pl.ANY),
        scratch_shapes=[
            pltpu.VMEM((S, D), BF16),
            pltpu.VMEM((D, 3 * D), BF16),
            pltpu.VMEM((D, D), BF16),
            pltpu.VMEM((D, F), BF16),
            pltpu.VMEM((D, F), BF16),
            pltpu.VMEM((F, D), BF16),
            pltpu.VMEM((S, D), BF16),
            pltpu.VMEM((S, D), BF16),
            pltpu.VMEM((H, QR, S), BF16),
            pltpu.VMEM((NTILE, S, 128), F32),
            pltpu.VMEM((H, VR, S), F32),
            pltpu.VMEM((H, VR, S), F32),
            pltpu.VMEM((2 * D, D), BF16),
            pltpu.VMEM((DH, NV + KB_PAD, 128), F32),
            pltpu.VMEM((DH, NV + KB_PAD, 128), F32),
            pltpu.VMEM((KQ * NQ, 128), F32),
            pltpu.VMEM((KQ * NQ, 128), F32),
            pltpu.VMEM((H, VR, S), F32),
            pltpu.VMEM((H, S), F32),
            pltpu.VMEM((3, 8, TQ), F32),
            pltpu.VMEM((S, D), F32),
            pltpu.VMEM((NQ + 1, NM, TQ), F32),
            pltpu.VMEM((2 * NQ, NV, TQ), F32),
            pltpu.VMEM((S, D), F32),
            pltpu.VMEM((UR, HG), F32),
            pltpu.VMEM((UR, HG), F32),
            pltpu.VMEM((S, D), F32),
            pltpu.SMEM((H + VA,), jnp.int32),
            pltpu.SemaphoreType.DMA((NX + 7 + NFR,)),
        ],
        compiler_params=pltpu.CompilerParams(vmem_limit_bytes=120 * 1024 * 1024),
    )(A_x.reshape(S, D), A_wqkv, A_wo, B_w_gate, B_w_up, B_w_down)
    return out.reshape(1, S, D)
```

```python
import math

import jax
import jax.numpy as jnp
import jax.experimental.pallas as pl
import jax.experimental.pallas.tpu as pltpu

S, D, F = 2048, 640, 1536
H, DH = 32, 20
VR = 24
QR = 32
NG = D // 128
NTILE = 2 * NG - 1
NT_DIMS = (((1,), (1,)), ((), ()))
NN_DIMS = (((1,), (0,)), ((), ()))
QSCALE = (DH ** -0.5) * math.log2(math.e)
F32 = jnp.float32
BF16 = jnp.bfloat16

SHIFT = 64.0
L_MIN = 2.0 ** -80
L_MAX = 2.0 ** 80
V_MAX = 2.0 ** 40

TQ = 512
CK = 128
SC = 128
FR = 256
PB = 128
FK = 128
NV = 384
KB_PAD = 8
HG = 768
UR = 128
NFUSE = F // HG
VA = 2
GRP = 32
WD = 256
VS = 480
XB = [0, 3, 9, 16]
XW = {2: [1], 8: [2]}
WAIT_B, T_POS = 8, 9
NX = len(XB) - 1
PIN_OFF, N_FREE, PIN_FRAC, PIN_TIME = 32, 3, 0.75, 0.72
DENSE_FIRST, DENSE_LAST, ACT_DELAY, N_EARLY = 1, 60, 2, 48

NQ = S // TQ
NT = TQ // 128
NC = S // CK
NFR = S // FR
NM = S - NV
KQ = -(-NM // (8 * NQ)) * 8
ROW_BOUNDS = [8 * ((NM // 8) * c // NC) for c in range(NC + 1)]
ITEMS = [(ju, kb, tt) for ju in range(NQ) for tt in range(NT) for kb in range(NV // (8 * VA))]


def _head_tile(h):
    lo = h * DH
    g0, g1 = lo // 128, (lo + DH - 1) // 128
    return g0 if g0 == g1 else NG + g0


NH = HG // 128


def _out_pieces(nk):
    out = []
    k0 = 0
    while nk - k0 >= 4:
        out += [(k0, k0 + 4, n, n + 1) for n in range(NG)]
        k0 += 4
    rem = nk - k0
    if rem:
        step = 4 // rem
        out += [(k0, nk, n, min(n + step, NG)) for n in range(0, NG, step)]
    return out


K4 = [("k4", i) for i in range(0, 2 * NH, 4)]
GU = [("gu", i) for i in range(2 * NH)]
DOWN = [("down", b) for b in _out_pieces(NH)]
DENSE = K4 + GU + DOWN


def _piece_time(p):
    kind, a = p
    if kind == "k4":
        return UR * min(4, 2 * NH - a) // 4
    if kind == "gu":
        return UR
    return UR * (a[1] - a[0]) * (a[3] - a[2]) // 4


DENSE_AT = {}
_first, _last = DENSE_FIRST, DENSE_LAST
for _p in range(len(DENSE)):
    DENSE_AT.setdefault(_first + (_p * (_last - _first)) // (len(DENSE) - 1), []).append(DENSE[_p])


def _pin_positions():
    n = len(ITEMS) - N_FREE
    total = NQ * NM + NQ * NC * VR + sum(_piece_time(p) for p in DENSE) - PIN_OFF
    pos = []
    for i in range(n):
        fr = (i + 1) / n
        if fr <= PIN_FRAC:
            t = fr / PIN_FRAC * PIN_TIME
        else:
            t = PIN_TIME + (fr - PIN_FRAC) / (1 - PIN_FRAC) * (1 - PIN_TIME)
        pos.append(max(0, (PIN_OFF + int(t * total)) // 8 * 8 - 8))
    return pos


PIN_POS = _pin_positions()


def _kernel(x_hbm, wqkv_hbm, wo_hbm, wg_hbm, wu_hbm, wd_hbm, out_hbm,
            x_ref, wqkv_ref, wo_ref, wg_ref, wu_ref, wd_ref, o_ref,
            xn_ref, qc_ref, k_ref, vt_ref, ot_ref, wt_ref,
            kba_ref, kbb_ref, kra_ref, krb_ref, qf_ref, kn_ref, lm_ref, ap_ref,
            s_ref, sv_ref, xf_ref, ha_ref, hb_ref, aw_ref, tile_ref, sems):
    def x_copy(r):
        rows = pl.ds(XB[r] * SC, (XB[r + 1] - XB[r]) * SC)
        return pltpu.make_async_copy(x_hbm.at[rows, :], x_ref.at[rows, :], sems.at[r])

    def w_copy(i):
        cols = pl.ds(i * D, D)
        return pltpu.make_async_copy(wqkv_hbm.at[:, cols], wqkv_ref.at[:, cols], sems.at[NX + i])

    late = [pltpu.make_async_copy(src, dst, sems.at[NX + 3 + i])
            for i, (src, dst) in enumerate([(wo_hbm, wo_ref), (wg_hbm, wg_ref), (wu_hbm, wu_ref), (wd_hbm, wd_ref)])]

    def out_copy(rows, r):
        return pltpu.make_async_copy(o_ref.at[rows, :], out_hbm.at[rows, :], sems.at[NX + 7 + r])

    x_copy(0).start()
    w_copy(1).start()
    for r in range(1, NX):
        x_copy(r).start()
    w_copy(0).start()
    w_copy(2).start()
    for h in range(H):
        tile_ref[h] = _head_tile(h)
    for a in range(VA):
        tile_ref[H + a] = 128 + a
    lm_ref[0] = jnp.full((8, TQ), 1.0, F32)
    lm_ref[1] = jnp.full((8, TQ), 1.0, F32)
    lm_ref[2] = jnp.zeros((8, TQ), F32)

    e_row = jax.lax.broadcasted_iota(jnp.int32, (H, D), 0)
    e_col = jax.lax.broadcasted_iota(jnp.int32, (H, D), 1)
    head_sel = jnp.where((e_col >= e_row * DH) & (e_col < (e_row + 1) * DH), 1.0, 0.0).astype(BF16)

    def layernorm(s):
        rows = pl.ds(s * SC, SC)
        x = x_ref[rows, :].astype(F32)
        mu = jnp.mean(x, axis=-1, keepdims=True)
        xc = x - mu
        var = jnp.mean(xc * xc, axis=-1, keepdims=True)
        xn = (xc * jax.lax.rsqrt(var + 1e-5)).astype(BF16)
        xn_ref[rows, :] = xn
        xf_ref[rows, :] = xn.astype(F32)

    def knorm(s, kk2):
        kn_ref[:, pl.ds(s * SC, SC)] = jax.lax.dot_general(head_sel, kk2, NT_DIMS, preferred_element_type=F32)

    def kproj(s):
        rows = pl.ds(s * SC, SC)
        kk = jnp.dot(xn_ref[rows, :], wqkv_ref[:, D:2 * D], preferred_element_type=F32)
        kk = kk.astype(BF16).astype(F32)
        lane = jax.lax.broadcasted_iota(jnp.int32, (SC, 128), 1)
        tiles = [kk[:, g * 128:(g + 1) * 128] for g in range(NG)]
        tiles += [jnp.where(lane >= 64, tiles[g], tiles[g + 1]) for g in range(NG - 1)]
        for g, tl in enumerate(tiles):
            k_ref[g, rows, :] = tl
        return (kk * kk).astype(BF16)

    n_sub = S // SC
    per = XB[1]
    x_copy(0).wait()
    for s in range(per):
        layernorm(s)
    w_copy(1).wait()
    prev = None
    for s in range(n_sub):
        for r in XW.get(s, []):
            x_copy(r).wait()
        if s == WAIT_B:
            w_copy(0).wait()
            w_copy(2).wait()
            for c in late:
                c.start()
        if per <= s + 1 < n_sub:
            layernorm(s + 1)
        if s == T_POS:
            wt_ref[0:D, :] = wqkv_ref[:, 0:D].astype(F32).T.astype(BF16)
            wt_ref[D:2 * D, :] = wqkv_ref[:, 2 * D:3 * D].astype(F32).T.astype(BF16)
        kk2 = kproj(s)
        if prev is not None:
            knorm(s - 1, prev)
        prev = kk2
    knorm(n_sub - 1, prev)
    kmax2 = jnp.max(kn_ref[...], axis=1, keepdims=True)

    def gen_kb(h, dst, d0, n):
        kv = k_ref[tile_ref[h], NM:S, :]
        for i in range(n):
            ln = (h * DH + d0 + i) % 128
            dst[d0 + i, 0:NV, :] = jnp.take_along_axis(kv, jnp.full((NV, 128), ln, jnp.int32), axis=1)

    def rotated_k(h, rows, n):
        kr = pltpu.roll(k_ref[tile_ref[h], rows, :], (D - h * DH) % 128, 1)
        lane = jax.lax.broadcasted_iota(jnp.int32, (n, 128), 1)
        return jnp.where(lane == DH, 1.0, kr)

    def scores(kc, qc):
        qm = jnp.concatenate([qc, jnp.zeros((128 - QR, TQ), BF16)], axis=0)
        return jax.lax.dot_general(kc, qm, NN_DIMS, preferred_element_type=F32)

    def qvproj(r, carry):
        rows = pl.ds(pl.multiple_of(r * TQ, TQ), TQ)
        xn = xn_ref[rows, :]
        qt = jax.lax.dot_general(wt_ref[0:D, :], xn, NT_DIMS, preferred_element_type=F32)
        qf = (qt * QSCALE).astype(BF16).astype(F32)
        vt0 = jax.lax.dot_general(wt_ref[D:D + VS, :], xn, NT_DIMS, preferred_element_type=F32)
        qn2 = jnp.dot(head_sel, (qf * qf).astype(BF16), preferred_element_type=F32)
        vt1 = jax.lax.dot_general(wt_ref[D + VS:2 * D, :], xn, NT_DIMS, preferred_element_type=F32)
        vt = jnp.concatenate([vt0, vt1], axis=0)
        lm_ref[2] = jnp.maximum(lm_ref[2], jnp.max(jnp.abs(vt).reshape(D // 8, 8, TQ), axis=0))
        negm = (SHIFT - jnp.sqrt(qn2 * kmax2)).astype(BF16).astype(F32)
        sub = jax.lax.broadcasted_iota(jnp.int32, (VR - DH, TQ), 0)
        tail = jnp.where(sub == 0, 1.0, 0.0).astype(F32)
        zpad = jnp.zeros((QR - VR, TQ), F32)
        for h in range(H):
            blk = jnp.concatenate([qf[h * DH:(h + 1) * DH, :], tail * negm[h:h + 1, :]], axis=0)
            qf_ref[h, :, rows] = blk
            qc_ref[h, :, rows] = jnp.concatenate([blk, zpad], axis=0).astype(BF16)
            vt_ref[h, 0:DH, rows] = vt[h * DH:(h + 1) * DH, :]
            vt_ref[h, DH:VR, rows] = tail
        lane = jax.lax.broadcasted_iota(jnp.int32, (S, 128), 1)
        s0 = scores(jnp.where(lane == DH, 1.0, k_ref[0]), qc_ref[0, :, rows])
        s_ref[r] = s0[0:NM]
        sv_ref[r] = s0[NM:S]
        gen_kb(1, kbb_ref, r * (DH // NQ), DH // NQ)
        krows = pl.ds(pl.multiple_of(r * KQ, 8), KQ)
        krb_ref[krows, :] = rotated_k(1, krows, KQ)
        return carry

    jax.lax.fori_loop(0, NQ, qvproj, 0)

    def activation(g, u):
        hg = 0.5 * g
        return (hg * (1.0 + jnp.tanh(hg))) * u

    def head_body(par, hq, hs, filler=None):
        kb_src, kb_dst = ((kba_ref, kbb_ref), (kbb_ref, kba_ref))[par]
        kr_src, kr_dst = ((kra_ref, krb_ref), (krb_ref, kra_ref))[par]
        h_dst, h_src = ((ha_ref, hb_ref), (hb_ref, ha_ref))[par]
        lane8 = jax.lax.broadcasted_iota(jnp.int32, (8, 128), 1)
        keep = [lane8 < tile_ref[H + a] for a in range(VA)]
        qrows = {}
        st = dict(done=0, t=0)

        def vpu_item(ju, kb_i, tt):
            tile = ju * NT + tt
            if tile not in qrows:
                blk = qf_ref[hq, :, tile * 128:(tile + 1) * 128]
                qrows[tile] = [jnp.broadcast_to(blk[i:i + 1, :], (GRP, 128)) for i in range(DH + 1)]
            g, o = divmod(kb_i * 8 * VA, GRP)
            if (tile, g) not in qrows:
                keys = slice(g * GRP, (g + 1) * GRP)
                q = qrows[tile]
                acc = q[DH]
                for d in range(DH):
                    acc = acc + kb_src[d, keys, :] * q[d]
                sv_ref[par * NQ + ju, keys, tt * 128:(tt + 1) * 128] = acc
                qrows[(tile, g)] = acc
            return qrows[(tile, g)][o:o + 8 * VA, :]

        def pinned(lhs, dur=None):
            n = lhs.shape[0]
            dur = n if dur is None else dur
            groups = [lhs[r:r + 8, :] for r in range(0, n, 8)]
            while st["done"] < len(PIN_POS) and PIN_POS[st["done"]] < st["t"] + dur:
                res = vpu_item(*ITEMS[st["done"]])
                gi = (PIN_POS[st["done"]] - st["t"]) // 8
                g0 = groups[gi][:, 0:128]
                for a in range(VA):
                    g0 = jnp.where(keep[a], g0, res[a * 8:(a + 1) * 8])
                groups[gi] = g0 if lhs.shape[1] == 128 else jnp.concatenate([g0, groups[gi][:, 128:]], axis=1)
                st["done"] += 1
            st["t"] += dur
            return jnp.concatenate(groups, axis=0)

        acts = []
        k4 = {}

        def wtile(i, k0, k1):
            n, w = divmod(i, 2)
            return (wg_ref, wu_ref)[w][k0:k1, par * HG + n * 128:par * HG + (n + 1) * 128]

        def dense(p):
            kind, a = p
            rows = pl.ds(pl.multiple_of((hq // NFUSE) * UR, UR), UR)
            if kind == "k4":
                ids = list(range(a, min(a + 4, 2 * NH)))
                lhs = pinned(xf_ref[rows, 512:640], _piece_time(p))
                w = jnp.concatenate([wtile(i, 512, 640) for i in ids], axis=1)
                res = jax.lax.dot_general(lhs, w, NN_DIMS, preferred_element_type=F32)
                for o, i in enumerate(ids):
                    k4[i] = res[:, o * 128:(o + 1) * 128]
            elif kind == "gu":
                lhs = pinned(xf_ref[rows, 0:512])
                k4[a] = jax.lax.dot_general(lhs, wtile(a, 0, 512), NN_DIMS, preferred_element_type=F32) + k4[a]
                if a % 2 == 1:
                    acts.append([ACT_DELAY, a // 2, k4[a - 1], k4[a]])
            else:
                down_piece(hs, 1 - par, a, pinned(h_src[:, a[0] * 128:a[1] * 128], _piece_time(p)))

        def tick():
            for a in list(acts):
                a[0] -= 1
                if a[0] <= 0:
                    h_dst[:, a[1] * 128:(a[1] + 1) * 128] = activation(a[2], a[3])
                    acts.pop(0)

        for j in range(NQ):
            js = (j + 1) % NQ
            src = s_ref.at[js if js else NQ * (1 - par)]
            dst = s_ref.at[j if j else NQ * par]
            vsrc = sv_ref.at[(1 - par) * NQ + js]
            if hq is not None:
                qc = qc_ref[hq, :, j * TQ:(j + 1) * TQ]
            acc_o = None
            for c in range(NC):
                lo, hi = c * CK, (c + 1) * CK
                parts = []
                if lo < NM:
                    parts.append(src[lo:min(hi, NM), :])
                if hi > NM:
                    parts.append(vsrc[max(lo, NM) - NM:hi - NM, :])
                sv = parts[0] if len(parts) == 1 else jnp.concatenate(parts, axis=0)
                vl = vt_ref[hs, :, lo:hi]
                pv = jnp.dot(pinned(vl) if hq is not None else vl, jnp.exp2(sv), preferred_element_type=F32)
                acc_o = pv if c == 0 else acc_o + pv
                if c == NC - 1:
                    lrows = acc_o[VR - 8:VR, :]
                    lm_ref[0] = jnp.minimum(lm_ref[0], lrows)
                    lm_ref[1] = jnp.maximum(lm_ref[1], lrows)
                    ot_ref[hs, :, js * TQ:(js + 1) * TQ] = acc_o
                if hq is not None:
                    r0, r1 = ROW_BOUNDS[c], ROW_BOUNDS[c + 1]
                    dst[r0:r1, :] = scores(pinned(kr_src[r0:r1, :]), qc)
                    tick()
                    for p in DENSE_AT.get(j * NC + c, []):
                        dense(p)
                    if c == 1:
                        hn = jnp.minimum(hq + 1, H - 1)
                        gen_kb(hn, kb_dst, j * (DH // NQ), DH // NQ)
                        kr_dst[j * KQ:(j + 1) * KQ, :] = rotated_k(hn, slice(j * KQ, (j + 1) * KQ), KQ)
                if filler is not None:
                    filler(j * NC + c)
        if hq is not None:
            assert not acts
            for it in ITEMS[st["done"]:]:
                vpu_item(*it)

    def down_piece(u, g, blk, hval):
        k0, k1, n0, n1 = blk
        if isinstance(u, int):
            rows = slice((u // NFUSE) * UR, (u // NFUSE + 1) * UR)
        else:
            rows = pl.ds(pl.multiple_of((u // NFUSE) * UR, UR), UR)
        cols = slice(n0 * 128, n1 * 128)
        y = jax.lax.dot_general(hval, wd_ref[g * HG + k0 * 128:g * HG + k1 * 128, cols], NN_DIMS,
                                preferred_element_type=F32)
        ap_ref[rows, cols] = y if (g == 0 and k0 == 0) else ap_ref[rows, cols] + y

    for c in late:
        c.wait()
    xn0 = xn_ref[0:UR, :]
    ha_ref[...] = activation(jnp.dot(xn0, wg_ref[:, 0:HG], preferred_element_type=F32),
                             jnp.dot(xn0, wu_ref[:, 0:HG], preferred_element_type=F32))

    def att(i, carry):
        @pl.when(i % 2 == 0)
        def _():
            head_body(0, i, i - 1)

        @pl.when(i % 2 == 1)
        def _():
            head_body(1, i, i - 1)
        return carry

    jax.lax.fori_loop(1, H, att, 0)

    def normalized(h, rows):
        return ot_ref[h, 0:DH, rows] / ot_ref[h, DH:DH + 1, rows]

    def wo_lhs(rows):
        ot = jnp.concatenate([normalized(h, rows) for h in range(-(-WD // DH))], axis=0)[0:WD, :]
        return ot.T.astype(BF16)

    lhs_cache = {}
    jobs = [("down", blk) for _, blk in DOWN] + [(b, blk) for b in range(S // PB) for blk in _out_pieces(WD // 128)]
    n_early = N_EARLY

    def run_job(job):
        b, blk = job
        k0, k1, n0, n1 = blk
        if b == "down":
            down_piece(H - 1, (H - 1) % 2, blk, hb_ref[:, k0 * 128:k1 * 128])
            return
        rows = slice(b * PB, (b + 1) * PB)
        if b not in lhs_cache:
            lhs_cache[b] = wo_lhs(rows)
        assert k0 == 0 and k1 * 128 == WD
        aw_ref[rows, n0 * 128:n1 * 128] = jnp.dot(lhs_cache[b], wo_ref[0:WD, n0 * 128:n1 * 128],
                                                  preferred_element_type=F32)

    def filler(k):
        for i in range(k * n_early // (NQ * NC), (k + 1) * n_early // (NQ * NC)):
            run_job(jobs[i])

    head_body(H % 2, None, H - 1, filler=filler)
    for job in jobs[n_early:]:
        run_job(job)

    lr = DH - (VR - 8)
    safe = ((jnp.min(lm_ref[0, lr:lr + 1, :]) >= L_MIN) & (jnp.max(lm_ref[1, lr:lr + 1, :]) <= L_MAX)
            & (jnp.max(lm_ref[2]) <= V_MAX))

    @pl.when(jnp.logical_not(safe))
    def _():
        def exact_unit(u, carry):
            h = u // NQ
            cols = pl.ds(pl.multiple_of((u % NQ) * TQ, TQ), TQ)
            idx = jax.lax.broadcasted_iota(jnp.int32, (QR, TQ), 0)
            qc = jnp.where(idx < DH, qc_ref[h, :, cols].astype(F32), 0.0).astype(BF16)

            def chunk(c, st):
                m, acc = st
                rows = pl.ds(pl.multiple_of(c * FK, FK), FK)
                s = scores(rotated_k(h, rows, FK), qc)
                m_new = jnp.maximum(m, jnp.max(s, axis=0, keepdims=True))
                p = jnp.exp2(s - m_new)
                acc = acc * jnp.exp2(m - m_new) + jnp.dot(vt_ref[h, :, rows], p, preferred_element_type=F32)
                return m_new, acc

            m0 = jnp.max(scores(rotated_k(h, slice(0, 8), 8), qc), axis=0, keepdims=True)
            _, acc = jax.lax.fori_loop(0, S // FK, chunk, (m0, jnp.zeros((VR, TQ), F32)))
            ot_ref[h, :, cols] = acc
            return carry

        jax.lax.fori_loop(0, H * NQ, exact_unit, 0)

        def redo(b, carry):
            rows = pl.ds(pl.multiple_of(b * PB, PB), PB)
            aw_ref[rows, :] = jnp.dot(wo_lhs(rows), wo_ref[0:WD, :], preferred_element_type=F32)
            return carry

        jax.lax.fori_loop(0, S // PB, redo, 0)

    h0 = WD // DH
    for r in range(NFR):
        rows = pl.ds(r * FR, FR)
        ot = jnp.concatenate([normalized(h, rows) for h in range(h0, H)], axis=0)[WD - h0 * DH:, :]
        acc = x_ref[rows, :].astype(F32) + ap_ref[rows, :] + aw_ref[rows, :]
        attn = jnp.dot(ot.T.astype(BF16), wo_ref[WD:D, :], preferred_element_type=F32)
        o_ref[rows, :] = (acc + attn).astype(o_ref.dtype)
        out_copy(rows, r).start()
    for r in range(NFR):
        out_copy(pl.ds(r * FR, FR), r).wait()


@jax.jit
def pallas_parallel_sum__softmax_full_mha__swiglu_ffn__prompt_kernel(
    A_x: jax.Array,
    A_wqkv: jax.Array,
    A_wo: jax.Array,
    B_x: jax.Array,
    B_w_gate: jax.Array,
    B_w_up: jax.Array,
    B_w_down: jax.Array,
):
    out = pl.pallas_call(
        _kernel,
        out_shape=jax.ShapeDtypeStruct((S, D), BF16),
        in_specs=[pl.BlockSpec(memory_space=pl.ANY)] * 6,
        out_specs=pl.BlockSpec(memory_space=pl.ANY),
        scratch_shapes=[
            pltpu.VMEM((S, D), BF16),
            pltpu.VMEM((D, 3 * D), BF16),
            pltpu.VMEM((D, D), BF16),
            pltpu.VMEM((D, F), BF16),
            pltpu.VMEM((D, F), BF16),
            pltpu.VMEM((F, D), BF16),
            pltpu.VMEM((S, D), BF16),
            pltpu.VMEM((S, D), BF16),
            pltpu.VMEM((H, QR, S), BF16),
            pltpu.VMEM((NTILE, S, 128), F32),
            pltpu.VMEM((H, VR, S), F32),
            pltpu.VMEM((H, VR, S), F32),
            pltpu.VMEM((2 * D, D), BF16),
            pltpu.VMEM((DH, NV + KB_PAD, 128), F32),
            pltpu.VMEM((DH, NV + KB_PAD, 128), F32),
            pltpu.VMEM((KQ * NQ, 128), F32),
            pltpu.VMEM((KQ * NQ, 128), F32),
            pltpu.VMEM((H, VR, S), F32),
            pltpu.VMEM((H, S), F32),
            pltpu.VMEM((3, 8, TQ), F32),
            pltpu.VMEM((S, D), F32),
            pltpu.VMEM((NQ + 1, NM, TQ), F32),
            pltpu.VMEM((2 * NQ, NV, TQ), F32),
            pltpu.VMEM((S, D), F32),
            pltpu.VMEM((UR, HG), F32),
            pltpu.VMEM((UR, HG), F32),
            pltpu.VMEM((S, D), F32),
            pltpu.SMEM((H + VA,), jnp.int32),
            pltpu.SemaphoreType.DMA((NX + 7 + NFR,)),
        ],
        compiler_params=pltpu.CompilerParams(vmem_limit_bytes=120 * 1024 * 1024),
    )(A_x.reshape(S, D), A_wqkv, A_wo, B_w_gate, B_w_up, B_w_down)
    return out.reshape(1, S, D)
```
